```python
import jax
import jax.numpy as jnp

def _softmax(x, axis=-1):
    return jax.nn.softmax(x, axis=axis)
def _gelu(x):
    return jax.nn.gelu(x, approximate=True)
def _silu(x):
    return jax.nn.silu(x)
def _sigmoid(x):
    return jax.nn.sigmoid(x)
def _layernorm(x, axis=-1, eps=1e-5):
    m = jnp.mean(x, axis=axis, keepdims=True)
    v = jnp.var(x, axis=axis, keepdims=True)
    return (x - m) / jnp.sqrt(v + eps)
def _scatter_add(tgt, idx, src, axis=0):
    return tgt.at[idx].add(src)
def _segment_sum(src, seg, n):
    return jax.ops.segment_sum(src, seg, n)
class _Rng:
    def __init__(self, key):
        self._k = key
    def _next(self):
        self._k, sub = jax.random.split(self._k)
        return sub
    def normal(self, shape):
        return jax.random.normal(self._next(), shape, dtype=jnp.bfloat16)
    def randint(self, lo, hi, shape):
        return jax.random.randint(self._next(), shape, lo, hi, dtype=jnp.int32)
    def uniform(self, shape, lo=0.0, hi=1.0):
        return jax.random.uniform(self._next(), shape, jnp.bfloat16, lo, hi)
    def permutation(self, n):
        return jax.random.permutation(self._next(), n)


kernel_name = 'sequential_preLN__sliding_block__glu_gated_glu__prompt'

def _fwd_setup_inputs():
    _rng = _Rng(jax.random.key(int.from_bytes(__import__("os").urandom(4), "little")))
    _w = (lambda a: (lambda t: t.astype(jnp.bfloat16) if jnp.issubdtype(t.dtype, jnp.floating) else t)(jnp.asarray(a)))
    def _A_setup():
        B, S, D = 1, 2048, 512
        return {
            "x": _w((lambda *s: _rng.normal(s) * 0.05)(B, S, D)),
            "wqkv": _w((lambda *s: _rng.normal(s) * 0.05)(D, 3 * D)),
            "wo": _w((lambda *s: _rng.normal(s) * 0.05)(D, D)),
        }
    _A_in = _A_setup()

    def _B_setup():
        B, S, D, F = 1, 2048, 512, 1376
        return {
            "x": _w((lambda *s: _rng.normal(s) * 0.05)(B, S, D)),
            "w_gate": _w((lambda *s: _rng.normal(s) * 0.05)(D, F)),
            "w_up": _w((lambda *s: _rng.normal(s) * 0.05)(D, F)),
            "w_down": _w((lambda *s: _rng.normal(s) * 0.05)(F, D)),
        }
    _B_in = _B_setup()

    return {
        "A_x": _A_in["x"],
        "A_wqkv": _A_in["wqkv"],
        "A_wo": _A_in["wo"],
        "B_x": _B_in["x"],
        "B_w_gate": _B_in["w_gate"],
        "B_w_up": _B_in["w_up"],
        "B_w_down": _B_in["w_down"],
    }

def _fwd_reference(A_x, A_wqkv, A_wo, B_x, B_w_gate, B_w_up, B_w_down):
    def _A_ref(x, wqkv, wo):
        B, S, D = x.shape
        H = 32; Dh = D // H; W = 256
        qkv = (lambda x, *d: x.transpose(*d))((x @ wqkv).reshape(B, S, 3, H, Dh), 2, 0, 3, 1, 4)
        q, k, v = qkv[0], qkv[1], qkv[2]
        scores = jnp.einsum("bhqd,bhkd->bhqk", q, k) * (Dh ** -0.5)
        idx = jnp.arange(S)
        mask = (idx[:, None] - idx[None, :] >= 0) & (idx[:, None] - idx[None, :] < W)
        scores = jnp.where(mask[None, None], scores, -1e9)
        p = _softmax(scores, axis=-1)
        o = jnp.einsum("bhqk,bhkd->bhqd", p, v)
        return (lambda x, *d: x.transpose(*d))(o, 0, 2, 1, 3).reshape(B, S, D) @ wo

    def _B_ref(x, w_gate, w_up, w_down):
        g = jnp.einsum("bsd,df->bsf", x, w_gate)
        u = jnp.einsum("bsd,df->bsf", x, w_up)
        h = _sigmoid(g) * u
        return jnp.einsum("bsf,fd->bsd", h, w_down)

    x = A_x
    h = x + _A_ref(_layernorm(x, axis=-1), A_wqkv, A_wo)
    h2 = h + _B_ref(_layernorm(h, axis=-1), B_w_gate, B_w_up, B_w_down)
    return h2


def setup_inputs():
    _inp = _fwd_setup_inputs()
    _gk = jax.random.fold_in(jax.random.key(int.from_bytes(__import__("os").urandom(4), "little")), 2**31 - 1)
    _shapes = [[1, 2048, 512]]
    _dtypes = ['bfloat16']
    _gks = jax.random.split(_gk, len(_shapes))
    _gs = [jax.random.normal(k, s, dtype=jnp.dtype(d)) * 0.05 for k, s, d in zip(_gks, _shapes, _dtypes)]
    _inp["grad_out"] = _gs[0]
    return _inp

def reference(A_x, A_wqkv, A_wo, B_w_gate, B_w_up, B_w_down, B_x, grad_out):
    _const = dict(B_x=B_x)
    def _f(*_d):
        return _fwd_reference(**{'A_x': _d[0], 'A_wqkv': _d[1], 'A_wo': _d[2], 'B_w_gate': _d[3], 'B_w_up': _d[4], 'B_w_down': _d[5], **_const})
    _out, _vjp = jax.vjp(_f, A_x, A_wqkv, A_wo, B_w_gate, B_w_up, B_w_down)
    _grads = _vjp(grad_out)
    _out0 = jnp.asarray(_out)
    return (_out0, *[jnp.asarray(_g) for _g in _grads])
```

```python
import jax
import jax.numpy as jnp
from jax import lax
import jax.experimental.pallas as pl
import jax.experimental.pallas.tpu as pltpu

S, D, F, DH = 2048, 512, 1376, 16
T = 128
NT = S // T
NG = D // T
RB = 256
QS = 0.25 * 1.4426950408889634
LN2 = 0.6931471805599453
EPS = 1e-5
bf, f32 = jnp.bfloat16, jnp.float32


def _nn(a, b):
    return jnp.dot(a, b, preferred_element_type=f32)


def _nt(a, b):
    return lax.dot_general(a, b, (((1,), (1,)), ((), ())), preferred_element_type=f32)


def _tn(a, b):
    return lax.dot_general(a, b, (((0,), (0,)), ((), ())), preferred_element_type=f32)


def _ln(x):
    m = jnp.mean(x, axis=-1, keepdims=True)
    c = x - m
    r = lax.rsqrt(jnp.mean(c * c, axis=-1, keepdims=True) + EPS)
    return c * r, r


def _ln_bwd(dy, y, r):
    return r * (dy - jnp.mean(dy, axis=-1, keepdims=True)
                - y * jnp.mean(dy * y, axis=-1, keepdims=True))


def _head_w(wt, hh):
    parts = []
    if hh > 0:
        parts.append(jnp.zeros((DH * hh, T), bf))
    parts.append(wt)
    if hh < 7:
        parts.append(jnp.zeros((DH * (7 - hh), T), bf))
    return jnp.concatenate(parts, axis=0)


def _kernel(x_ref, wqkv_ref, wo_ref, wg_ref, wu_ref, wd_ref, do_ref,
            out_ref, dx_ref, dwqkv_ref, dwo_ref, dwg_ref, dwu_ref, dwd_ref,
            xn_s, qT_s, k_s, kT_s, v_s, vT_s, oT_s, p_s, il_s, dl_s, dh_s, dhb_s):
    TPB = RB // T

    def p1(b, _):
        r0 = pl.multiple_of(b * RB, RB)
        xn, _r = _ln(x_ref[pl.ds(r0, RB), :].astype(f32))
        xn = xn.astype(bf)
        xn_s[pl.ds(r0, RB), :] = xn
        qkv = _nn(xn, wqkv_ref[...])
        q = (qkv[:, :D] * QS).astype(bf)
        k = qkv[:, D:2 * D].astype(bf)
        v = qkv[:, 2 * D:].astype(bf)
        for g in range(NG):
            k_s[g, pl.ds(r0, RB), :] = k[:, g * T:(g + 1) * T]
            v_s[g, pl.ds(r0, RB), :] = v[:, g * T:(g + 1) * T]
        for t in range(TPB):
            qT_s[b * TPB + t] = q[t * T:(t + 1) * T].T
            kT_s[b * TPB + t] = k[t * T:(t + 1) * T].T
            vT_s[b * TPB + t] = v[t * T:(t + 1) * T].T
        return 0
    lax.fori_loop(0, S // RB, p1, 0)

    def win(ref, g, i, n):
        return ref[g, pl.ds(pl.multiple_of((i - (n - 1)) * T, T), n * T), :]

    def tri():
        return (lax.broadcasted_iota(jnp.int32, (T, T), 0)
                <= lax.broadcasted_iota(jnp.int32, (T, T), 1))

    def att_fwd(i, g, n):
        m = tri()
        kw = win(k_s, g, i, n)
        for hh in range(8):
            c0 = pl.multiple_of(g * T + hh * DH, DH)
            rows = pl.ds(c0, DH)
            s = _nn(kw, _head_w(qT_s[i, rows, :], hh))
            if n == 3:
                s = jnp.concatenate([jnp.where(m, s[2 * T:], s[:T]), s[T:2 * T]], axis=0)
            elif n == 2:
                s = jnp.concatenate([jnp.where(m, s[T:], -1e30), s[:T]], axis=0)
            else:
                s = jnp.where(m, s, -1e30)
            e = jnp.exp2(s - jnp.max(s, axis=0, keepdims=True))
            il = 1.0 / jnp.sum(e, axis=0, keepdims=True)
            il_s[i, g * 8 + hh] = il
            eb = e.astype(bf)
            ee = eb[:T]
            if n == 3:
                p_s[i, g * 8 + hh] = eb
                z = jnp.zeros_like(ee)
                o = (_nn(vT_s[i, rows, :], jnp.where(m, ee, z))
                     + _nn(vT_s[i - 1, rows, :], eb[T:])
                     + _nn(vT_s[i - 2, rows, :], jnp.where(m, z, ee)))
            elif n == 2:
                p_s[i, g * 8 + hh] = eb
                o = _nn(vT_s[i, rows, :], ee) + _nn(vT_s[i - 1, rows, :], eb[T:])
            else:
                p_s[i, g * 8 + hh, :T] = eb
                o = _nn(vT_s[i, rows, :], ee)
            oT_s[i, rows, :] = (o * il).astype(bf)

    def over_tiles(fn):
        def per_g(g, _):
            fn(0, g, 1)
            fn(1, g, 2)

            def per_i(i, _):
                fn(i, g, 3)
                return 0
            lax.fori_loop(2, NT, per_i, 0)
            return 0
        lax.fori_loop(0, NG, per_g, 0)
    over_tiles(att_fwd)

    def ffn(hnT_s, act_s, dg_s, du_s):
        def p3(b, _):
            r0 = pl.multiple_of(b * RB, RB)
            rs = pl.ds(r0, RB)
            oT = jnp.concatenate([oT_s[b * TPB + t] for t in range(TPB)], axis=1)
            h = x_ref[rs, :].astype(f32) + _tn(oT, wo_ref[...])
            hn, r = _ln(h)
            hb = hn.astype(bf)
            hnT_s[b] = hb.T
            sg = jax.nn.sigmoid(_nn(hb, wg_ref[...]))
            u = _nn(hb, wu_ref[...])
            act = (sg * u).astype(bf)
            act_s[rs, :] = act
            out_ref[rs, :] = (h + _nn(act, wd_ref[...])).astype(bf)
            do = do_ref[rs, :]
            da = _nt(do, wd_ref[...])
            du = da * sg
            dg = (du * u * (1.0 - sg)).astype(bf)
            du = du.astype(bf)
            dg_s[rs, :] = dg
            du_s[rs, :] = du
            dhn = _nt(dg, wg_ref[...]) + _nt(du, wu_ref[...])
            dh = do.astype(f32) + _ln_bwd(dhn, hn, r)
            dh_s[rs, :] = dh
            dhb = dh.astype(bf)
            dhb_s[rs, :] = dhb
            dOT = _nt(wo_ref[...], dhb)
            dd = dOT * oT.astype(f32)
            for t in range(TPB):
                i = b * TPB + t
                for hd in range(32):
                    il = il_s[i, hd]
                    sl = (slice(hd * DH, (hd + 1) * DH), slice(t * T, (t + 1) * T))
                    dl_s[i, hd] = jnp.sum(dd[sl], axis=0, keepdims=True) * il
                    qT_dO[i, sl[0], :] = (dOT[sl] * il).astype(bf)
            return 0
        lax.fori_loop(0, S // RB, p3, 0)

        hnT = jnp.concatenate([hnT_s[b] for b in range(S // RB)], axis=1)
        dwg_ref[...] = _nn(hnT, dg_s[...]).astype(bf)
        dwu_ref[...] = _nn(hnT, du_s[...]).astype(bf)
        dwd_ref[...] = _tn(act_s[...], do_ref[...]).astype(bf)
        for g in range(NG):
            oTg = jnp.concatenate([oT_s[i, g * T:(g + 1) * T, :] for i in range(NT)], axis=1)
            dwo_ref[g * T:(g + 1) * T, :] = _nn(oTg, dhb_s[...]).astype(bf)

    qT_dO = vT_s
    pl.run_scoped(ffn, pltpu.VMEM((S // RB, D, RB), bf), pltpu.VMEM((S, F), bf),
                  pltpu.VMEM((S, F), bf), pltpu.VMEM((S, F), bf))

    def bwd(dT_s):
        dT_s[...] = jnp.zeros_like(dT_s)

        def att_bwd(i, g, n):
            m = tri()
            vw = win(v_s, g, i, n)
            for hh in range(8):
                c0 = pl.multiple_of(g * T + hh * DH, DH)
                rows = pl.ds(c0, DH)
                doh = qT_dO[i, rows, :]
                qh = qT_s[i, rows, :]
                dp = _nn(vw, _head_w(doh, hh))
                if n == 3:
                    dp = jnp.concatenate([jnp.where(m, dp[2 * T:], dp[:T]), dp[T:2 * T]], axis=0)
                elif n == 2:
                    dp = jnp.concatenate([dp[T:], dp[:T]], axis=0)
                eb = p_s[i, g * 8 + hh] if n > 1 else p_s[i, g * 8 + hh, :T]
                ds = (eb.astype(f32) * (dp - dl_s[i, g * 8 + hh])).astype(bf)
                ee, de = eb[:T], ds[:T]
                if n == 3:
                    z = jnp.zeros_like(ee)
                    tiles = [(i, jnp.where(m, ee, z), jnp.where(m, de, z)),
                             (i - 1, eb[T:], ds[T:]),
                             (i - 2, jnp.where(m, z, ee), jnp.where(m, z, de))]
                elif n == 2:
                    tiles = [(i, ee, de), (i - 1, eb[T:], ds[T:])]
                else:
                    tiles = [(i, ee, de)]
                dq = None
                for j, pj, dj in tiles:
                    a = _nn(kT_s[j, rows, :], dj)
                    dq = a if dq is None else dq + a
                    dT_s[j, pl.ds(D + c0, DH), :] += _nt(qh, dj)
                    dT_s[j, pl.ds(2 * D + c0, DH), :] += _nt(doh, pj)
                dT_s[i, rows, :] = dq * 0.25
        over_tiles(att_bwd)

        def p5a(i, _):
            oT_s[i] = dT_s[i, :D, :].astype(bf)
            qT_s[i] = (dT_s[i, D:2 * D, :] * LN2).astype(bf)
            kT_s[i] = dT_s[i, 2 * D:, :].astype(bf)
            return 0
        lax.fori_loop(0, NT, p5a, 0)
        src = (oT_s, qT_s, kT_s)

        def p5(b, _):
            r0 = pl.multiple_of(b * RB, RB)
            rs = pl.ds(r0, RB)
            dT = jnp.concatenate(
                [jnp.concatenate([s_[b * TPB + t] for t in range(TPB)], axis=1) for s_ in src], axis=0)
            dxn = _nn(wqkv_ref[...], dT).T
            y, r = _ln(x_ref[rs, :].astype(f32))
            dx_ref[rs, :] = (dh_s[rs, :] + _ln_bwd(dxn, y, r)).astype(bf)
            return 0
        lax.fori_loop(0, S // RB, p5, 0)
        for c in range(3):
            for g in range(NG):
                dTg = jnp.concatenate([src[c][i, g * T:(g + 1) * T, :] for i in range(NT)], axis=1)
                dwqkv_ref[:, c * D + g * T:c * D + (g + 1) * T] = _nn(dTg, xn_s[...]).T.astype(bf)
    pl.run_scoped(bwd, pltpu.VMEM((NT, 3 * D, T), f32))


@jax.jit
def pallas_sequential_preLN__sliding_block__glu_gated_glu__prompt_kernel(
    A_x, A_wqkv, A_wo, B_x, B_w_gate, B_w_up, B_w_down, grad_out,
):
    sd = jax.ShapeDtypeStruct
    outs = pl.pallas_call(
        _kernel,
        out_shape=(sd((S, D), bf), sd((S, D), bf), sd((D, 3 * D), bf), sd((D, D), bf),
                   sd((D, F), bf), sd((D, F), bf), sd((F, D), bf)),
        scratch_shapes=[
            pltpu.VMEM((S, D), bf),
            pltpu.VMEM((NT, D, T), bf),
            pltpu.VMEM((NG, S, T), bf),
            pltpu.VMEM((NT, D, T), bf),
            pltpu.VMEM((NG, S, T), bf),
            pltpu.VMEM((NT, D, T), bf),
            pltpu.VMEM((NT, D, T), bf),
            pltpu.VMEM((NT, 32, 2 * T, T), bf),
            pltpu.VMEM((NT, 32, 1, T), f32),
            pltpu.VMEM((NT, 32, 1, T), f32),
            pltpu.VMEM((S, D), f32),
            pltpu.VMEM((S, D), bf),
        ],
        compiler_params=pltpu.CompilerParams(vmem_limit_bytes=127 * 2**20),
    )(A_x[0], A_wqkv, A_wo, B_w_gate, B_w_up, B_w_down, grad_out[0])
    return (outs[0][None], outs[1][None]) + tuple(outs[2:])
```

```python
import jax
import jax.numpy as jnp
from jax import lax
import jax.experimental.pallas as pl
import jax.experimental.pallas.tpu as pltpu

S, D, F, DH = 2048, 512, 1376, 16
T = 128
NT = S // T
NG = D // T
RB = 512
QS = 0.25 * 1.4426950408889634
LN2 = 0.6931471805599453
EPS = 1e-5
bf, f32 = jnp.bfloat16, jnp.float32


def _nn(a, b):
    return jnp.dot(a, b, preferred_element_type=f32)


def _nt(a, b):
    return lax.dot_general(a, b, (((1,), (1,)), ((), ())), preferred_element_type=f32)


def _tn(a, b):
    return lax.dot_general(a, b, (((0,), (0,)), ((), ())), preferred_element_type=f32)


def _ln(x):
    m = jnp.mean(x, axis=-1, keepdims=True)
    c = x - m
    r = lax.rsqrt(jnp.mean(c * c, axis=-1, keepdims=True) + EPS)
    return c * r, r


def _ln_bwd(dy, y, r):
    return r * (dy - jnp.mean(dy, axis=-1, keepdims=True)
                - y * jnp.mean(dy * y, axis=-1, keepdims=True))


def _head_w(wt, hh):
    parts = []
    if hh > 0:
        parts.append(jnp.zeros((DH * hh, T), bf))
    parts.append(wt)
    if hh < 7:
        parts.append(jnp.zeros((DH * (7 - hh), T), bf))
    return jnp.concatenate(parts, axis=0)


def _kernel(*refs):
    hin, hout, vin, vout = refs[:7], refs[7:14], refs[14:21], refs[21:28]
    cin = [pltpu.make_async_copy(hin[j], vin[j], refs[28].at[j]) for j in range(7)]
    cout = [pltpu.make_async_copy(vout[j], hout[j], refs[29].at[j]) for j in range(7)]
    cin[0].start()
    cin[1].start()
    _body(cin, cout, *vin, *vout, *refs[30:])
    for c in cout:
        c.wait()


def _body(cin, cout, x_ref, wqkv_ref, wo_ref, wg_ref, wu_ref, wd_ref, do_ref,
            out_ref, dx_ref, dwqkv_ref, dwo_ref, dwg_ref, dwu_ref, dwd_ref,
            xn_s, qT_s, k_s, kT_s, v_s, vT_s, oT_s, p_s, il_s, dl_s, dh_s, dhb_s, mb_s, s_s, tr_s):
    TPB = RB // T

    def p1(b, _):
        r0 = pl.multiple_of(b * RB, RB)
        xn, _r = _ln(x_ref[pl.ds(r0, RB), :].astype(f32))
        xn = xn.astype(bf)
        xn_s[pl.ds(r0, RB), :] = xn
        qkv = _nn(xn, wqkv_ref[...])
        q = (qkv[:, :D] * QS).astype(bf)
        k = qkv[:, D:2 * D].astype(bf)
        v = qkv[:, 2 * D:].astype(bf)
        for g in range(NG):
            k_s[g, pl.ds(r0, RB), :] = k[:, g * T:(g + 1) * T]
            v_s[g, pl.ds(r0, RB), :] = v[:, g * T:(g + 1) * T]
        for t in range(TPB):
            qT_s[b * TPB + t] = q[t * T:(t + 1) * T].T
            kT_s[b * TPB + t] = k[t * T:(t + 1) * T].T
            vT_s[b * TPB + t] = v[t * T:(t + 1) * T].T
        return 0
    cin[0].wait()
    cin[1].wait()
    for c in cin[2:]:
        c.start()
    with jax.named_scope('p1'):
        lax.fori_loop(0, S // RB, p1, 0)

    def win(ref, g, i, n):
        return ref[g, pl.ds(pl.multiple_of((i - (n - 1)) * T, T), n * T), :]

    def tri():
        return (lax.broadcasted_iota(jnp.int32, (T, T), 0)
                <= lax.broadcasted_iota(jnp.int32, (T, T), 1))

    mb_s[...] = pltpu.bitcast(jnp.where(tri(), -1, 0).astype(jnp.int16), jnp.int32)

    def split(x):
        xi = pltpu.bitcast(x, jnp.int32)
        lo = xi & mb_s[...]
        return pltpu.bitcast(lo, bf), pltpu.bitcast(xi ^ lo, bf)

    def tp(x, hh, slot):
        n = hh * 6 + slot
        tr_s[n] = x.T
        return tr_s[n]

    def hrows(g, hh):
        return pl.ds(pl.multiple_of(g * T + hh * DH, DH), DH)

    def scores(i, g, n, h0):
        m = tri()
        kw = win(k_s, g, i, n)
        ss = []
        for hh in range(h0, h0 + 4):
            s = _nn(kw, _head_w(qT_s[i, hrows(g, hh), :], hh))
            if n == 3:
                s = jnp.concatenate([jnp.where(m, s[2 * T:], s[:T]), s[T:2 * T]], axis=0)
            elif n == 2:
                s = jnp.concatenate([jnp.where(m, s[T:], -1e30), s[:T]], axis=0)
            else:
                s = jnp.where(m, s, -1e30)
            ss.append(s)
        return ss

    def att_fwd(i, g, n):
        if n == 3:
            @pl.when(i == 2)
            def _():
                for hh, s in enumerate(scores(i, g, n, 0)):
                    s_s[hh] = s
        for h0 in (0, 4):
            if h0 == 0:
                nxt = scores(i, g, n, 4)
                if n < 3:
                    cur = scores(i, g, n, 0)
                else:
                    cur = [s_s[hh] for hh in range(4)]
            else:
                cur = nxt
                if n == 3:
                    for hh, s in enumerate(scores(jnp.minimum(i + 1, NT - 1), g, n, 0)):
                        s_s[hh] = s
            es, ils = [], []
            for hh in range(h0, h0 + 4):
                s = cur[hh - h0]
                e = jnp.exp2(s - jnp.max(s, axis=0, keepdims=True))
                il = 1.0 / jnp.sum(e, axis=0, keepdims=True)
                il_s[i, g * 8 + hh] = il
                eb = e.astype(bf)
                if n > 1:
                    p_s[i, g * 8 + hh] = eb
                else:
                    p_s[i, g * 8 + hh, :T] = eb
                es.append(eb)
                ils.append(il)
            for hh, eb, il in zip(range(h0, h0 + 4), es, ils):
                rows = hrows(g, hh)
                if n == 3:
                    lo, hi = split(eb[:T])
                    o = (_nn(vT_s[i - 1, rows, :], eb[T:]) + _nn(vT_s[i, rows, :], lo)
                         + _nn(vT_s[i - 2, rows, :], hi))
                elif n == 2:
                    o = _nn(vT_s[i, rows, :], eb[:T]) + _nn(vT_s[i - 1, rows, :], eb[T:])
                else:
                    o = _nn(vT_s[i, rows, :], eb)
                oT_s[i, rows, :] = (o * il).astype(bf)

    def over_tiles(fn):
        def per_g(g, _):
            fn(0, g, 1)
            fn(1, g, 2)

            def per_i(i, _):
                fn(i, g, 3)
                return 0
            lax.fori_loop(2, NT, per_i, 0)
            return 0
        lax.fori_loop(0, NG, per_g, 0)
    with jax.named_scope('att_fwd'):
        over_tiles(att_fwd)

    def ffn(hn_s, act_s, dg_s, du_s):
        def p3(b, _):
            r0 = pl.multiple_of(b * RB, RB)
            rs = pl.ds(r0, RB)
            oT = jnp.concatenate([oT_s[b * TPB + t] for t in range(TPB)], axis=1)
            h = x_ref[rs, :].astype(f32) + _tn(oT, wo_ref[...])
            hn, r = _ln(h)
            hb = hn.astype(bf)
            hn_s[rs, :] = hb
            sg = jax.nn.sigmoid(_nt(hb, wg_ref[...]))
            u = _nt(hb, wu_ref[...])
            act = (sg * u).astype(bf)
            act_s[rs, :] = act
            out_ref[rs, :] = (h + _nn(act, wd_ref[...])).astype(bf)
            do = do_ref[rs, :]
            da = _nt(do, wd_ref[...])
            du = da * sg
            dg = (du * u * (1.0 - sg)).astype(bf)
            du = du.astype(bf)
            dg_s[rs, :] = dg
            du_s[rs, :] = du
            dhn = _nn(dg, wg_ref[...]) + _nn(du, wu_ref[...])
            dh = do.astype(f32) + _ln_bwd(dhn, hn, r)
            dh_s[rs, :] = dh
            dhb = dh.astype(bf)
            dhb_s[rs, :] = dhb
            dOT = _nt(wo_ref[...], dhb)
            dd = dOT * oT.astype(f32)
            for t in range(TPB):
                i = b * TPB + t
                for hd in range(32):
                    il = il_s[i, hd]
                    sl = (slice(hd * DH, (hd + 1) * DH), slice(t * T, (t + 1) * T))
                    dl_s[i, hd] = jnp.sum(dd[sl], axis=0, keepdims=True) * il
                    qT_dO[i, sl[0], :] = (dOT[sl] * il).astype(bf)
            return 0
        with jax.named_scope('p3'):
            lax.fori_loop(0, S // RB, p3, 0)
        cout[0].start()
        with jax.named_scope('pw_gu'):
            dwg_ref[...] = _tn(dg_s[...], hn_s[...]).astype(bf)
            cout[4].start()
            dwu_ref[...] = _tn(du_s[...], hn_s[...]).astype(bf)
            cout[5].start()
        with jax.named_scope('pw_d'):
            dwd_ref[...] = _tn(act_s[...], do_ref[...]).astype(bf)
            cout[6].start()
        with jax.named_scope('pw_o'):
            for g in range(NG):
                oTg = jnp.concatenate([oT_s[i, g * T:(g + 1) * T, :] for i in range(NT)], axis=1)
                dwo_ref[g * T:(g + 1) * T, :] = _nn(oTg, dhb_s[...]).astype(bf)

    for c in cin[2:]:
        c.wait()
    qT_dO = vT_s
    pl.run_scoped(ffn, pltpu.VMEM((S, D), bf), pltpu.VMEM((S, F), bf),
                  pltpu.VMEM((S, F), bf), pltpu.VMEM((S, F), bf))

    cout[3].start()

    def bwd(dT_s):
        with jax.named_scope('pz'):
            dT_s[...] = jnp.zeros_like(dT_s)

        def att_bwd(i, g, n):
            m = tri()
            vw = win(v_s, g, i, n)
            dps = [_nn(vw, _head_w(qT_dO[i, hrows(g, hh), :], hh)) for hh in range(8)]
            for h0 in (0, 4):
                tl = []
                for hh in range(h0, h0 + 4):
                    dp = dps[hh]
                    if n == 3:
                        dp = jnp.concatenate([jnp.where(m, dp[2 * T:], dp[:T]), dp[T:2 * T]], axis=0)
                    elif n == 2:
                        dp = jnp.concatenate([dp[T:], dp[:T]], axis=0)
                    eb = p_s[i, g * 8 + hh] if n > 1 else p_s[i, g * 8 + hh, :T]
                    ds = (eb.astype(f32) * (dp - dl_s[i, g * 8 + hh])).astype(bf)
                    ee, de = eb[:T], ds[:T]
                    if n == 3:
                        (e0, e2), (d0, d2) = split(ee), split(de)
                        tl.append([(i, e0, d0), (i - 1, eb[T:], ds[T:]), (i - 2, e2, d2)])
                    elif n == 2:
                        tl.append([(i, ee, de), (i - 1, eb[T:], ds[T:])])
                    else:
                        tl.append([(i, ee, de)])
                for hh, tiles in zip(range(h0, h0 + 4), tl):
                    rows = hrows(g, hh)
                    dq = None
                    for j, pj, dj in tiles:
                        a = _nn(kT_s[j, rows, :], dj)
                        dq = a if dq is None else dq + a
                    dT_s[i, rows, :] = dq * 0.25
                for hh, tiles in zip(range(h0, h0 + 4), tl):
                    c0 = pl.multiple_of(g * T + hh * DH, DH)
                    doh = qT_dO[i, hrows(g, hh), :]
                    qh = qT_s[i, hrows(g, hh), :]
                    for t, (j, pj, dj) in enumerate(tiles):
                        dT_s[j, pl.ds(D + c0, DH), :] += _nn(qh, dj.T)
                        dT_s[j, pl.ds(2 * D + c0, DH), :] += _nn(doh, tp(pj, hh, 3 + t))
        with jax.named_scope('att_bwd'):
            over_tiles(att_bwd)

        def p5a(i, _):
            oT_s[i] = dT_s[i, :D, :].astype(bf)
            qT_s[i] = (dT_s[i, D:2 * D, :] * LN2).astype(bf)
            kT_s[i] = dT_s[i, 2 * D:, :].astype(bf)
            return 0
        with jax.named_scope('p5a'):
            lax.fori_loop(0, NT, p5a, 0)
        src = (oT_s, qT_s, kT_s)
        with jax.named_scope('pw_qkv'):
            for c in range(3):
                for g in range(NG):
                    dTg = jnp.concatenate([src[c][i, g * T:(g + 1) * T, :] for i in range(NT)], axis=1)
                    dwqkv_ref[:, c * D + g * T:c * D + (g + 1) * T] = _nn(dTg, xn_s[...]).T.astype(bf)
        cout[2].start()

        def p5(b, _):
            r0 = pl.multiple_of(b * RB, RB)
            rs = pl.ds(r0, RB)
            dT = jnp.concatenate(
                [jnp.concatenate([s_[b * TPB + t] for t in range(TPB)], axis=1) for s_ in src], axis=0)
            dxn = _nn(wqkv_ref[...], dT).T
            y, r = _ln(x_ref[rs, :].astype(f32))
            dx_ref[rs, :] = (dh_s[rs, :] + _ln_bwd(dxn, y, r)).astype(bf)
            return 0
        with jax.named_scope('p5'):
            lax.fori_loop(0, S // RB, p5, 0)
        cout[1].start()
    pl.run_scoped(bwd, pltpu.VMEM((NT, 3 * D, T), f32))


@jax.jit
def pallas_sequential_preLN__sliding_block__glu_gated_glu__prompt_kernel(
    A_x, A_wqkv, A_wo, B_x, B_w_gate, B_w_up, B_w_down, grad_out,
):
    sd = jax.ShapeDtypeStruct
    FD = sd((F, D), bf)
    ins = (A_x[0], A_wqkv, A_wo, B_w_gate.T, B_w_up.T, B_w_down, grad_out[0])
    out_shape = (sd((S, D), bf), sd((S, D), bf), sd((D, 3 * D), bf), sd((D, D), bf), FD, FD, FD)
    hbm = pl.BlockSpec(memory_space=pl.ANY)
    outs = pl.pallas_call(
        _kernel,
        out_shape=out_shape,
        in_specs=[hbm] * 7,
        out_specs=[hbm] * 7,
        scratch_shapes=[pltpu.VMEM(a.shape, bf) for a in ins + out_shape] + [
            pltpu.SemaphoreType.DMA((7,)),
            pltpu.SemaphoreType.DMA((7,)),
            pltpu.VMEM((S, D), bf),
            pltpu.VMEM((NT, D, T), bf),
            pltpu.VMEM((NG, S, T), bf),
            pltpu.VMEM((NT, D, T), bf),
            pltpu.VMEM((NG, S, T), bf),
            pltpu.VMEM((NT, D, T), bf),
            pltpu.VMEM((NT, D, T), bf),
            pltpu.VMEM((NT, 32, 2 * T, T), bf),
            pltpu.VMEM((NT, 32, 1, T), f32),
            pltpu.VMEM((NT, 32, 1, T), f32),
            pltpu.VMEM((S, D), f32),
            pltpu.VMEM((S, D), bf),
            pltpu.VMEM((T // 2, T), jnp.int32),
            pltpu.VMEM((4, 2 * T, T), f32),
            pltpu.VMEM((48, T, T), bf),
        ],
        compiler_params=pltpu.CompilerParams(vmem_limit_bytes=127 * 2**20),
    )(*ins)
    return (outs[0][None], outs[1][None], outs[2], outs[3], outs[4].T, outs[5].T, outs[6])
```
